```python
import os as _os
_os.environ.setdefault("JAX_PLATFORMS", "cpu")
import jax
import jax.numpy as jnp

def _softmax(x, axis=-1):
    return jax.nn.softmax(x, axis=axis)
def _gelu(x):
    return jax.nn.gelu(x, approximate=True)
def _silu(x):
    return jax.nn.silu(x)
def _sigmoid(x):
    return jax.nn.sigmoid(x)
def _layernorm(x, axis=-1, eps=1e-5):
    m = jnp.mean(x, axis=axis, keepdims=True)
    v = jnp.var(x, axis=axis, keepdims=True)
    return (x - m) / jnp.sqrt(v + eps)
def _scatter_add(tgt, idx, src, axis=0):
    return tgt.at[idx].add(src)
def _segment_sum(src, seg, n):
    return jax.ops.segment_sum(src, seg, n)
class _Rng:
    def __init__(self, key):
        self._k = key
    def _next(self):
        self._k, sub = jax.random.split(self._k)
        return sub
    def normal(self, shape):
        return jax.random.normal(self._next(), shape, dtype=jnp.bfloat16)
    def randint(self, lo, hi, shape):
        return jax.random.randint(self._next(), shape, lo, hi, dtype=jnp.int32)
    def uniform(self, shape, lo=0.0, hi=1.0):
        return jax.random.uniform(self._next(), shape, jnp.bfloat16, lo, hi)
    def permutation(self, n):
        return jax.random.permutation(self._next(), n)


kernel_name = 'gated_mix__compressed_kv_cla__linear_attn_block__prompt'

def setup_inputs():
    _rng = _Rng(jax.random.key(int.from_bytes(__import__("os").urandom(4), "little")))
    _w = (lambda a: (lambda t: t.astype(jnp.bfloat16) if jnp.issubdtype(t.dtype, jnp.floating) else t)(jnp.asarray(a)))
    def _A_setup():
        B, H, Sq, Sk, D, M = 1, 16, 2048, 2048, 256, 448
        Dc = 4 * D
        return {
            "x": _w((lambda *s: _rng.normal(s) * 0.05)(B, Sq, M)),
            "c_kv": _w((lambda *s: _rng.normal(s) * 0.8)(B, Sk, Dc)),
            "w_q": _w((lambda *s: _rng.normal(s) * 3.2)(M, H, D) * (M ** -0.5)),
            "w_uk": _w((lambda *s: _rng.normal(s) * 3.2)(Dc, H, D) * (Dc ** -0.5)),
            "w_uv": _w((lambda *s: _rng.normal(s) * 0.8)(Dc, H, D) * (Dc ** -0.5)),
            "w_o": _w((lambda *s: _rng.normal(s) * 0.8)(H, D, M) * ((H * D) ** -0.5)),
        }
    _A_in = _A_setup()

    def _B_setup():
        B, S, D = 1, 2048, 448
        return {
            "x": _w((lambda *s: _rng.normal(s) * 0.05)(B, S, D)),
            "wqkv": _w((lambda *s: _rng.normal(s) * 1.6)(D, 3 * D)),
            "wo": _w((lambda *s: _rng.normal(s) * 0.4)(D, D)),
        }
    _B_in = _B_setup()

    return {
        "A_x": _A_in["x"],
        "A_c_kv": _A_in["c_kv"],
        "A_w_q": _A_in["w_q"],
        "A_w_uk": _A_in["w_uk"],
        "A_w_uv": _A_in["w_uv"],
        "A_w_o": _A_in["w_o"],
        "B_x": _B_in["x"],
        "B_wqkv": _B_in["wqkv"],
        "B_wo": _B_in["wo"],
        "gate_w": _w((lambda *s: _rng.normal(s) * 0.05)(448) * 16.0),
    }

def reference(A_x, A_c_kv, A_w_q, A_w_uk, A_w_uv, A_w_o, B_x, B_wqkv, B_wo, gate_w):
    def _A_ref(x, c_kv, w_q, w_uk, w_uv, w_o):
        B, Sq, M = x.shape[0], x.shape[1], x.shape[2]
        Sk = c_kv.shape[1]
        H, D = w_q.shape[1], w_q.shape[2]
        q = jnp.einsum("bqm,mhd->bhqd", x, w_q)
        k = jnp.einsum("bkc,chd->bhkd", c_kv, w_uk)
        v = jnp.einsum("bkc,chd->bhkd", c_kv, w_uv)
        scores = jnp.einsum("bhqd,bhkd->bhqk", q, k) * (D ** -0.5)
        off = Sk - Sq
        qi = jnp.arange(Sq)[:, None]
        kj = jnp.arange(Sk)[None, :]
        cmask = kj <= (qi + off)
        scores = jnp.where(cmask[None, None], scores, -1e9)
        p = _softmax(scores, axis=-1)
        ctx = jnp.einsum("bhqk,bhkd->bhqd", p, v)
        return jnp.einsum("bhqd,hdm->bqm", ctx, w_o)

    def _B_ref(x, wqkv, wo):
        B, S, D = x.shape
        H = 16; Dh = D // H
        qkv = (lambda x, *d: x.transpose(*d))((x @ wqkv).reshape(B, S, 3, H, Dh), 2, 0, 3, 1, 4)
        q, k, v = qkv[0], qkv[1], qkv[2]
        phi = lambda t: jnp.where(t > 0, t + 1, jnp.exp(t)) + 1e-6
        pq, pk = phi(q), phi(k)
        kv = jnp.einsum("bhsd,bhse->bhde", pk, v)
        z = jnp.einsum("bhsd->bhd", pk)
        num = jnp.einsum("bhqd,bhde->bhqe", pq, kv)
        den = jnp.einsum("bhqd,bhd->bhq", pq, z)[..., None] + 1e-6
        o = num / den
        return (lambda x, *d: x.transpose(*d))(o, 0, 2, 1, 3).reshape(B, S, D) @ wo

    x = A_x
    g = _sigmoid((x * gate_w).sum(-1, keepdims=True))
    a = _A_ref(x, A_c_kv, A_w_q, A_w_uk, A_w_uv, A_w_o)
    b = _B_ref(x, B_wqkv, B_wo)
    return g * a + (1 - g) * b
```

```python
import functools
import numpy as np
import jax
import jax.numpy as jnp
from jax import lax
import jax.experimental.pallas as pl
import jax.experimental.pallas.tpu as pltpu

bf16 = jnp.bfloat16
f32 = jnp.float32
S = 2048
M = 448
H = 16
D = 256
DC = 1024
DH = 28
LOG2E = 1.4426950408889634
N_ = (((1,), (0,)), ((), ()))
NT = (((1,), (1,)), ((), ()))
TN = (((0,), (0,)), ((), ()))


def _dot(a, b, dims=N_):
    return lax.dot_general(a, b, dims, preferred_element_type=f32)


def _kernel(xa_hbm, ckv_hbm, wq_hbm, wk_hbm, wv_hbm, wo_hbm, wqkv_hbm, bwo_hbm, gw_hbm,
            out_hbm,
            xaT_v, xa_v, ckv_v, wq_raw, wk_raw, wv_raw, wo_v, wqkv_v, bwo_v, gw_v,
            wqh, wkh, wvh, q_s, k_s, v_s, ctx_s, g_s, b_s, o_s, sems, *, cfg):
    def cp(src, dst, i):
        return pltpu.make_async_copy(src, dst, sems.at[i])
    c_wqkv = cp(wqkv_hbm, wqkv_v, 1)
    c_bwo = cp(bwo_hbm, bwo_v, 2)
    c_xa = cp(xa_hbm, xaT_v, 3)
    c_gw = cp(gw_hbm, gw_v, 4)
    c_ckv = [cp(ckv_hbm.at[:, 128 * k:128 * (k + 1)], ckv_v.at[k], 5 + k) for k in range(8)]
    c_wk = [cp(wk_hbm.at[:, 128 * t:128 * (t + 1)], wk_raw.at[t], 13 + t) for t in range(2)]
    c_wv = [cp(wv_hbm.at[:, 128 * t:128 * (t + 1)], wv_raw.at[t], 15 + t) for t in range(2)]
    c_wq = [cp(wq_hbm.at[:, 128 * t:128 * (t + 1)], wq_raw.at[t], 17 + t) for t in range(2)]
    c_wo = [cp(wo_hbm.at[:, :, 128 * t:128 * (t + 1)], wo_v.at[t], 19 + t) for t in range(2)]
    for c in [c_xa, c_wqkv, c_gw, c_bwo, *c_wq, *c_ckv, *c_wk, *c_wv, *c_wo]:
        c.start()

    def phi(t):
        return jnp.where(t > 0, t + 1.0, jnp.exp(t)) + 1e-6

    c_xa.wait()
    c_wqkv.wait()
    xbT = xaT_v[...]
    wq_b = wqkv_v[:, 0:M]
    wk_b = wqkv_v[:, M:2 * M]
    wv_b = wqkv_v[:, 2 * M:3 * M]
    pkT = phi(_dot(wk_b, xbT, TN))
    z = jnp.sum(pkT, axis=1, keepdims=True)
    t = _dot(pkT.astype(bf16), xbT, NT)
    kv = _dot(t.astype(bf16), wv_b)
    rh = lax.broadcasted_iota(jnp.int32, (M, M), 0) // DH
    ch = lax.broadcasted_iota(jnp.int32, (M, M), 1) // DH
    bd = rh == ch
    kv_bd = jnp.where(bd, kv, 0.0).astype(bf16)
    zbdT = jnp.where(bd, z, 0.0).astype(bf16)
    c_bwo.wait()
    kvw = _dot(kv_bd, bwo_v[...]).astype(bf16)
    pqT = phi(_dot(wq_b, xbT, TN))
    den = _dot(zbdT, pqT.astype(bf16), TN) + 1e-6
    pqn = (pqT / den).astype(bf16)
    b_s[...] = _dot(kvw, pqn, TN)

    c_gw.wait()
    gw = jnp.broadcast_to(gw_v[...].reshape(1, M), (16, M))
    logit = _dot(gw, xaT_v[...])
    g_s[...] = jax.nn.sigmoid(logit[0:8])
    xa = xaT_v[...].T
    for k in range(3):
        xa_v[k] = xa[:, 128 * k:128 * (k + 1)]
    xa_v[3] = jnp.concatenate([xa[:, 384:448], jnp.zeros((S, 64), bf16)], axis=1)

    def relayout(raw, dst, rows):
        for t in range(2):
            r32 = raw.at[t].bitcast(jnp.uint32)
            for j in range(8):
                w = r32[pl.ds(j, rows, stride=8), :]
                dst[2 * j, t, 0:rows] = pltpu.bitcast(w << 16, f32).astype(bf16)
                dst[2 * j + 1, t, 0:rows] = pltpu.bitcast(w & jnp.uint32(0xFFFF0000), f32).astype(bf16)

    for c in c_wq:
        c.wait()
    relayout(wq_raw, wqh, M)
    wqh[:, :, M:512, :] = jnp.zeros((H, 2, 512 - M, 128), bf16)
    for c in c_wk:
        c.wait()
    relayout(wk_raw, wkh, DC)
    for c in c_wv:
        c.wait()
    relayout(wv_raw, wvh, DC)
    for c in c_ckv:
        c.wait()

    BQ = cfg['bq']
    qscale = (D ** -0.5) * LOG2E

    def cat(ref, r0, r1):
        return jnp.concatenate([ref[0, r0:r1, :], ref[1, r0:r1, :]], axis=1)

    def head(h, carry):
        MC = cfg['mc']
        wk = jnp.concatenate([wkh[h, 0], wkh[h, 1]], axis=1)
        wv = jnp.concatenate([wvh[h, 0], wvh[h, 1]], axis=1)
        wq = jnp.concatenate([wqh[h, 0], wqh[h, 1]], axis=1)
        for m0 in range(0, S, MC):
            c = jnp.concatenate([ckv_v[k, m0:m0 + MC, :] for k in range(8)], axis=1)
            kk = _dot(c, wk).astype(bf16)
            k_s[0, m0:m0 + MC, :] = kk[:, :128]
            k_s[1, m0:m0 + MC, :] = kk[:, 128:]
            vv = _dot(c, wv).astype(bf16)
            v_s[0, m0:m0 + MC, :] = vv[:, :128]
            v_s[1, m0:m0 + MC, :] = vv[:, 128:]
            x = jnp.concatenate([xa_v[k, m0:m0 + MC, :] for k in range(4)], axis=1)
            qq = (_dot(x, wq) * qscale).astype(bf16)
            q_s[0, m0:m0 + MC, :] = qq[:, :128]
            q_s[1, m0:m0 + MC, :] = qq[:, 128:]

        tri = (lax.broadcasted_iota(jnp.int32, (128, 128), 0) >= lax.broadcasted_iota(jnp.int32, (128, 128), 1))
        NEG = -1e9 * LOG2E

        def qk(i):
            r0 = i * BQ
            nsub = BQ // 128
            q = cat(q_s, r0, r0 + BQ)
            parts = []
            if r0 > 0:
                parts.append((0, BQ, 0, r0, _dot(q, cat(k_s, 0, r0), NT)))
            for c in range(nsub):
                rs = c * 128
                s = _dot(q[rs:], cat(k_s, r0 + rs, r0 + rs + 128), NT)
                top = jnp.where(tri, s[:128], NEG)
                s = top if rs + 128 == BQ else jnp.concatenate([top, s[128:]], axis=0)
                parts.append((rs, BQ, r0 + rs, r0 + rs + 128, s))
            return parts

        def softmax_pv(i, parts):
            r0 = i * BQ
            nsub = BQ // 128
            for g in range(nsub):
                segs = [(c0, c1, s[g * 128 - rs:g * 128 - rs + 128]) for (rs, _, c0, c1, s) in parts if rs <= g * 128]
                sfull = jnp.concatenate([x[2] for x in segs], axis=1) if len(segs) > 1 else segs[0][2]
                m = jnp.max(sfull, axis=1, keepdims=True)
                p = jnp.exp2(sfull - m)
                l = jnp.sum(p, axis=1, keepdims=True)
                L = r0 + (g + 1) * 128
                o = _dot(p.astype(bf16), cat(v_s, 0, L))
                o = (o * (1.0 / l)).astype(bf16)
                ctx_s[2 * h, r0 + g * 128:r0 + (g + 1) * 128, :] = o[:, :128]
                ctx_s[2 * h + 1, r0 + g * 128:r0 + (g + 1) * 128, :] = o[:, 128:]

        nq = S // BQ
        if cfg['pipe']:
            prev = qk(0)
            for i in range(nq):
                nxt = qk(i + 1) if i + 1 < nq else None
                softmax_pv(i, prev)
                prev = nxt
        else:
            for i in range(nq):
                softmax_pv(i, qk(i))
        return carry

    lax.fori_loop(0, H, head, 0)

    for c in c_wo:
        c.wait()
    OC = cfg['oc']
    wo = jnp.concatenate([wo_v[t, h] for h in range(H) for t in range(2)], axis=1)
    outs = []
    for i, q0 in enumerate(range(0, S, OC)):
        rhs = jnp.concatenate([ctx_s[k, q0:q0 + OC, :] for k in range(2 * H)], axis=1)
        a = _dot(wo, rhs, NT)
        g = g_s[0:1, q0:q0 + OC]
        o_s[:, q0:q0 + OC] = (g * a + (1.0 - g) * b_s[:, q0:q0 + OC]).astype(bf16)
        d = pltpu.make_async_copy(o_s.at[:, q0:q0 + OC], out_hbm.at[:, q0:q0 + OC], sems.at[21 + i])
        d.start()
        outs.append(d)
    for d in outs:
        d.wait()


def _forward(cfg, A_x, A_c_kv, A_w_q, A_w_uk, A_w_uv, A_w_o, B_x, B_wqkv, B_wo, gate_w):
    xa = A_x.reshape(S, M).T
    ckv = A_c_kv.reshape(S, DC)
    wq = A_w_q.reshape(M * H, D)
    wk = A_w_uk.reshape(DC * H, D)
    wv = A_w_uv.reshape(DC * H, D)
    wo = jnp.transpose(A_w_o, (0, 2, 1))
    V = pltpu.VMEM
    scratch = [
        V((M, S), bf16), V((4, S, 128), bf16), V((8, S, 128), bf16), V((2, M * H, 128), bf16),
        V((2, DC * H, 128), bf16), V((2, DC * H, 128), bf16), V((2, H, M, 128), bf16),
        V((M, 3 * M), bf16), V((M, M), bf16), V((M,), bf16),
        V((H, 2, 512, 128), bf16), V((H, 2, DC, 128), bf16), V((H, 2, DC, 128), bf16),
        V((2, S, 128), bf16), V((2, S, 128), bf16), V((2, S, 128), bf16),
        V((2 * H, S, 128), bf16), V((8, S), f32), V((M, S), f32), V((M, S), bf16),
        pltpu.SemaphoreType.DMA((21 + S // cfg['oc'],)),
    ]
    out = pl.pallas_call(
        functools.partial(_kernel, cfg=cfg),
        out_shape=jax.ShapeDtypeStruct((M, S), bf16),
        in_specs=[pl.BlockSpec(memory_space=pl.ANY)] * 9,
        out_specs=pl.BlockSpec(memory_space=pl.ANY),
        scratch_shapes=scratch,
        compiler_params=pltpu.CompilerParams(vmem_limit_bytes=120 * 2 ** 20),
        name="gm_v2",
    )(xa, ckv, wq, wk, wv, wo, B_wqkv, B_wo, gate_w)
    return out.T.reshape(1, S, M)


DEFAULT = dict(bq=256, mc=512, oc=512, pipe=False)


_CFG = DEFAULT


@jax.jit
def pallas_gated_mix__compressed_kv_cla__linear_attn_block__prompt_kernel(
    A_x: jax.Array,
    A_c_kv: jax.Array,
    A_w_q: jax.Array,
    A_w_uk: jax.Array,
    A_w_uv: jax.Array,
    A_w_o: jax.Array,
    B_x: jax.Array,
    B_wqkv: jax.Array,
    B_wo: jax.Array,
    gate_w: jax.Array,
):
    return _forward(_CFG, A_x, A_c_kv, A_w_q, A_w_uk, A_w_uv, A_w_o, B_x, B_wqkv, B_wo, gate_w)
```

```python
import functools
import numpy as np
import jax
import jax.numpy as jnp
from jax import lax
import jax.experimental.pallas as pl
import jax.experimental.pallas.tpu as pltpu

bf16 = jnp.bfloat16
f32 = jnp.float32
S = 2048
M = 448
H = 16
D = 256
DC = 1024
DH = 28
LOG2E = 1.4426950408889634
N_ = (((1,), (0,)), ((), ()))
NT = (((1,), (1,)), ((), ()))
TN = (((0,), (0,)), ((), ()))


def _dot(a, b, dims=N_):
    return lax.dot_general(a, b, dims, preferred_element_type=f32)


def _kernel(xa_hbm, ckv_hbm, wq_hbm, wk_hbm, wv_hbm, wo_hbm, wqkv_hbm, bwo_hbm, gw_hbm,
            out_hbm,
            xaT_v, xa_v, ckv_v, wq_raw, wk_raw, wv_raw, wo_v, wqkv_v, bwo_v, gw_v,
            wqh, wkh, wvh, wq0, wk0, wv0, q_s, k_s, v_s, ctx_s, g_s, b_s, o_s, sems, *, cfg):
    def cp(src, dst, i):
        return pltpu.make_async_copy(src, dst, sems.at[i])
    c_wqkv = [cp(wqkv_hbm.at[:, a:b], wqkv_v.at[:, a:b], i) for i, (a, b) in enumerate([(384, 896), (0, 384), (896, 3 * M)])]
    c_bwo = cp(bwo_hbm, bwo_v, 21)
    c_xa = [cp(xa_hbm.at[:, a:a + 1024], xaT_v.at[0:M, a:a + 1024], 22 + a // 1024) for a in (0, 1024)]
    c_gw = cp(gw_hbm, gw_v, 4)
    c_ckv = [cp(ckv_hbm.at[:, 128 * k:128 * (k + 1)], ckv_v.at[k], 5 + k) for k in range(8)]
    c_wk = [cp(wk_hbm.at[:, 128 * t:128 * (t + 1)], wk_raw.at[t], 13 + t) for t in range(2)]
    c_wv = [cp(wv_hbm.at[:, 128 * t:128 * (t + 1)], wv_raw.at[t], 15 + t) for t in range(2)]
    c_wq = [cp(wq_hbm.at[:, 128 * t:128 * (t + 1)], wq_raw.at[t], 17 + t) for t in range(2)]
    c_wo = [cp(wo_hbm.at[:, :, 128 * t:128 * (t + 1)], wo_v.at[t], 19 + t) for t in range(2)]
    for c in [c_wqkv[0], c_xa[0], c_xa[1], c_wqkv[1], c_gw, c_wqkv[2], c_bwo, *c_wk, *c_ckv, *c_wv, *c_wq, *c_wo]:
        c.start()

    def relayout_pieces(raw, dst0, dst, rows, rc):
        def piece(j, t, r0, lo, hi):
            def run(zero):
                w = raw.at[t].bitcast(jnp.uint32)[pl.ds(8 * r0 + j, rc, stride=8), :]
                sh, msk = 16, jnp.uint32(0xFFFF0000)
                if zero is not None:
                    zero = jnp.concatenate([zero] * (rc // 8), axis=0)
                    sh, msk = zero + 16, zero | msk
                if lo is not None:
                    lo[r0:r0 + rc] = pltpu.bitcast(w << sh, f32).astype(bf16)
                if hi is not None:
                    hi[r0:r0 + rc] = pltpu.bitcast(w & msk, f32).astype(bf16)
            return run
        first = [piece(0, t, r0, dst0.at[t], None) for r0 in range(0, rows, rc) for t in range(2)]
        rest = [piece(j, t, r0, dst.at[2 * j, t] if j > 0 else None, dst.at[2 * j + 1, t])
                for j in range(8) for r0 in range(0, rows, rc) for t in range(2)]
        return first, rest

    def interleave(main, side):
        n = len(main)
        for i, f in enumerate(main):
            r = f()
            zero = None if r is None else (pltpu.bitcast(r[0:8, 0:128], jnp.uint32) >> 31) >> 1
            for s_ in side[i * len(side) // n:(i + 1) * len(side) // n]:
                s_(zero)

    def phi(t):
        return jnp.where(t > 0, t + 1.0, jnp.exp(t)) + 1e-6

    row16 = lax.broadcasted_iota(jnp.int32, (16, S), 0)
    xaT_v[M:M + 16, :] = jnp.where(row16 == 0, 1.0, 0.0).astype(bf16)
    c_wqkv[0].wait()
    c_xa[0].wait()
    wkT = wqkv_v[:, M:2 * M].T
    pk = []
    for i in range(2):
        if i == 1:
            for c in [c_xa[1], c_wqkv[1], c_gw, c_wqkv[2], c_bwo]:
                c.wait()
        pk.append(phi(_dot(wkT, xaT_v[0:M, 1024 * i:1024 * (i + 1)])).astype(bf16))
    pkT = jnp.concatenate(pk, axis=1)
    xT = xaT_v[0:M, :]
    pqT = phi(_dot(wqkv_v[:, 0:M], xT, TN))
    gw = jnp.broadcast_to(gw_v[...].reshape(1, M), (16, M))
    g_s[...] = jax.nn.sigmoid(_dot(gw, xT)[0:8])
    tT = _dot(xaT_v[...], pkT, NT)
    z = tT[M:M + 1, :]
    hh = lax.broadcasted_iota(jnp.int32, (16, M), 0)
    hd = lax.broadcasted_iota(jnp.int32, (16, M), 1) // DH
    zc = jnp.where(hh == hd, z, 0.0).astype(bf16)
    den = _dot(zc, pqT.astype(bf16)) + 1e-6
    rden = 1.0 / den
    rhi = rden.astype(bf16)
    rlo = (rden - rhi.astype(f32)).astype(bf16)
    eh = lax.broadcasted_iota(jnp.int32, (M, 32), 0) // DH
    ec = lax.broadcasted_iota(jnp.int32, (M, 32), 1) % 16
    rfull = _dot(jnp.where(eh == ec, 1.0, 0.0).astype(bf16), jnp.concatenate([rhi, rlo], axis=0))
    pqn = (pqT * rfull).astype(bf16)
    kvT = _dot(wqkv_v[:, 2 * M:3 * M], tT[0:M].astype(bf16), TN)
    rh = lax.broadcasted_iota(jnp.int32, (M, M), 0) // DH
    ch = lax.broadcasted_iota(jnp.int32, (M, M), 1) // DH
    kvT = jnp.where(rh == ch, kvT, 0.0).astype(bf16)
    kvwT = _dot(bwo_v[...], kvT, TN).astype(bf16)
    for c in c_wk:
        c.wait()
    first, rest = relayout_pieces(wk_raw, wk0, wkh, DC, cfg["rc"])

    def b_chunk(q0):
        def run():
            r = _dot(kvwT, pqn[:, q0:q0 + 256])
            b_s[:, q0:q0 + 256] = r
            return r
        return run
    interleave([b_chunk(q0) for q0 in range(0, S, 256)], first + rest)


    BQ = cfg['bq']
    MC = cfg['mc']
    qscale = (D ** -0.5) * LOG2E
    NEG = -1e9 * LOG2E

    def cat(ref, r0, r1):
        return jnp.concatenate([ref[0, r0:r1, :], ref[1, r0:r1, :]], axis=1)

    def put(ref, r0, r1, val):
        ref[0, r0:r1, :] = val[:, :128]
        ref[1, r0:r1, :] = val[:, 128:]

    def kv_proj(w_ref, dst, side=(), MC=MC):
        def chunk(m0):
            def run():
                c = jnp.concatenate([ckv_v[k, m0:m0 + MC, :] for k in range(8)], axis=1)
                w = jnp.concatenate([w_ref[0], w_ref[1]], axis=1)
                r = _dot(c, w)
                put(dst, m0, m0 + MC, r.astype(bf16))
                return r
            return run
        interleave([chunk(m0) for m0 in range(0, S, MC)], list(side))

    def q_proj(w_ref, side=(), MC=MC):
        def chunk(m0):
            def run():
                w = jnp.concatenate([w_ref[0], w_ref[1]], axis=1)
                x = jnp.concatenate([xa_v[k, m0:m0 + MC, :] for k in range(4)], axis=1)
                r = _dot(x, w) * qscale
                put(q_s, m0, m0 + MC, r.astype(bf16))
                return r
            return run
        interleave([chunk(m0) for m0 in range(0, S, MC)], list(side))

    def qk(i):
        tri = (lax.broadcasted_iota(jnp.int32, (128, 128), 0) >= lax.broadcasted_iota(jnp.int32, (128, 128), 1))
        r0 = i * BQ
        nsub = BQ // 128
        q = cat(q_s, r0, r0 + BQ)
        parts = []
        if r0 > 0:
            parts.append((0, _dot(q, cat(k_s, 0, r0), NT)))
        for c in range(nsub):
            rs = c * 128
            s = _dot(q[rs:], cat(k_s, r0 + rs, r0 + rs + 128), NT)
            top = jnp.where(tri, s[:128], NEG)
            s = top if rs + 128 == BQ else jnp.concatenate([top, s[128:]], axis=0)
            parts.append((rs, s))
        return parts

    def softmax_pv(h, i, parts):
        r0 = i * BQ
        nsub = BQ // 128
        for g in range(nsub):
            segs = [s[g * 128 - rs:g * 128 - rs + 128] for (rs, s) in parts if rs <= g * 128]
            sfull = jnp.concatenate(segs, axis=1) if len(segs) > 1 else segs[0]
            m = jnp.max(sfull, axis=1, keepdims=True)
            p = jnp.exp2(sfull - m)
            l = jnp.sum(p, axis=1, keepdims=True)
            L = r0 + (g + 1) * 128
            o = _dot(p.astype(bf16), cat(v_s, 0, L))
            r = pl.reciprocal(l, approx=True)
            r = r * (2.0 - l * r)
            o = (o * r).astype(bf16)
            ctx_s[2 * h, r0 + g * 128:r0 + (g + 1) * 128, :] = o[:, :128]
            ctx_s[2 * h + 1, r0 + g * 128:r0 + (g + 1) * 128, :] = o[:, 128:]

    def attention(h, fill_kq, fill_v):
        nq = S // BQ
        prev = qk(nq - 1)
        for i in reversed(range(nq)):
            nxt = qk(i - 1) if i > 0 else None
            fill_kq(i)
            softmax_pv(h, i, prev)
            fill_v(i)
            prev = nxt

    def proj_tile(w_ref, dst, i, isq=False):
        m0 = i * BQ
        w = jnp.concatenate([w_ref[0], w_ref[1]], axis=1)
        if isq:
            x = jnp.concatenate([xa_v[k, m0:m0 + BQ, :] for k in range(4)], axis=1)
            put(dst, m0, m0 + BQ, (_dot(x, w) * qscale).astype(bf16))
        else:
            c = jnp.concatenate([ckv_v[k, m0:m0 + BQ, :] for k in range(8)], axis=1)
            put(dst, m0, m0 + BQ, _dot(c, w).astype(bf16))

    def xpose(q0):
        def run(zero):
            xa = xaT_v[0:M, q0:q0 + 256].T
            for k in range(3):
                xa_v[k, q0:q0 + 256] = xa[:, 128 * k:128 * (k + 1)]
            xa_v[3, q0:q0 + 256] = jnp.concatenate([xa[:, 384:448], jnp.zeros((256, 64), bf16)], axis=1)
        return run

    for c in c_ckv:
        c.wait()
    kv_proj(wk0, k_s, [xpose(q0) for q0 in range(0, S, 256)], 256)
    for c in c_wv:
        c.wait()
    first, rest = relayout_pieces(wv_raw, wv0, wvh, DC, cfg["rc"])
    interleave([lambda: None], first)
    kv_proj(wv0, v_s, rest, cfg['mc0'])
    wqh[1:H, :, M:512, :] = jnp.zeros((H - 1, 2, 512 - M, 128), bf16)
    wq0[:, M:512, :] = jnp.zeros((2, 512 - M, 128), bf16)
    for c in c_wq:
        c.wait()
    first, rest = relayout_pieces(wq_raw, wq0, wqh, M, min(64, cfg["rc"]))
    interleave([lambda: None], first)
    q_proj(wq0, rest, cfg['mc0'])

    def head(h, carry):
        attention(h, lambda i: (proj_tile(wkh.at[h + 1], k_s, i), proj_tile(wqh.at[h + 1], q_s, i, True)),
                  lambda i: proj_tile(wvh.at[h + 1], v_s, i))
        return carry

    lax.fori_loop(0, H - 1, head, 0, unroll=cfg["unroll"])

    OC = cfg['oc']
    outs = []

    def out_proj(chunks, hs):
        wo = jnp.concatenate([wo_v[t, h] for h in hs for t in range(2)], axis=1)
        for i in chunks:
            q0 = i * OC
            rhs = jnp.concatenate([ctx_s[2 * h + t, q0:q0 + OC, :] for h in hs for t in range(2)], axis=1)
            yield i, _dot(wo, rhs, NT)

    nq = S // BQ
    nc = S // OC

    def partial_out(i):
        if i % (nq // nc) == 0:
            for ci, a in out_proj([i // (nq // nc)], range(H - 1)):
                q0 = ci * OC
                g = g_s[0:1, q0:q0 + OC]
                b_s[:, q0:q0 + OC] = g * a + (1.0 - g) * b_s[:, q0:q0 + OC]

    for c in c_wo:
        c.wait()
    attention(H - 1, partial_out, lambda i: None)
    for i, a in out_proj(range(S // OC), [H - 1]):
        q0 = i * OC
        g = g_s[0:1, q0:q0 + OC]
        o_s[:, q0:q0 + OC] = (g * a + b_s[:, q0:q0 + OC]).astype(bf16)
        d = pltpu.make_async_copy(o_s.at[:, q0:q0 + OC], out_hbm.at[:, q0:q0 + OC], sems.at[24 + i])
        d.start()
        outs.append(d)
    for d in outs:
        d.wait()


def _forward(cfg, A_x, A_c_kv, A_w_q, A_w_uk, A_w_uv, A_w_o, B_x, B_wqkv, B_wo, gate_w):
    xa = A_x.reshape(S, M).T
    ckv = A_c_kv.reshape(S, DC)
    wq = A_w_q.reshape(M * H, D)
    wk = A_w_uk.reshape(DC * H, D)
    wv = A_w_uv.reshape(DC * H, D)
    wo = jnp.transpose(A_w_o, (0, 2, 1))
    V = pltpu.VMEM
    scratch = [
        V((M + 16, S), bf16), V((4, S, 128), bf16), V((8, S, 128), bf16), V((2, M * H, 128), bf16),
        V((2, DC * H, 128), bf16), V((2, DC * H, 128), bf16), V((2, H, M, 128), bf16),
        V((M, 3 * M), bf16), V((M, M), bf16), V((M,), bf16),
        V((H, 2, 512, 128), bf16), V((H, 2, DC, 128), bf16), V((H, 2, DC, 128), bf16),
        V((2, 512, 128), bf16), V((2, DC, 128), bf16), V((2, DC, 128), bf16),
        V((2, S, 128), bf16), V((2, S, 128), bf16), V((2, S, 128), bf16),
        V((2 * H, S, 128), bf16), V((8, S), f32), V((M, S), f32), V((M, S), bf16),
        pltpu.SemaphoreType.DMA((24 + S // cfg['oc'],)),
    ]
    out = pl.pallas_call(
        functools.partial(_kernel, cfg=cfg),
        out_shape=jax.ShapeDtypeStruct((M, S), bf16),
        in_specs=[pl.BlockSpec(memory_space=pl.ANY)] * 9,
        out_specs=pl.BlockSpec(memory_space=pl.ANY),
        scratch_shapes=scratch,
        compiler_params=pltpu.CompilerParams(vmem_limit_bytes=120 * 2 ** 20),
        name="gm_v11",
    )(xa, ckv, wq, wk, wv, wo, B_wqkv, B_wo, gate_w)
    return out.T.reshape(1, S, M)


DEFAULT = dict(bq=128, mc=256, mc0=128, split=True, oc=256, rc=32, unroll=1)


_CFG = DEFAULT


@jax.jit
def pallas_gated_mix__compressed_kv_cla__linear_attn_block__prompt_kernel(
    A_x: jax.Array,
    A_c_kv: jax.Array,
    A_w_q: jax.Array,
    A_w_uk: jax.Array,
    A_w_uv: jax.Array,
    A_w_o: jax.Array,
    B_x: jax.Array,
    B_wqkv: jax.Array,
    B_wo: jax.Array,
    gate_w: jax.Array,
):
    return _forward(_CFG, A_x, A_c_kv, A_w_q, A_w_uk, A_w_uv, A_w_o, B_x, B_wqkv, B_wo, gate_w)
```
